```python
import jax
import jax.numpy as jnp

def _softmax(x, axis=-1):
    return jax.nn.softmax(x, axis=axis)

def _gelu(x):
    return jax.nn.gelu(x, approximate=True)

def _silu(x):
    return jax.nn.silu(x)

def _sigmoid(x):
    return jax.nn.sigmoid(x)

def _layernorm(x, axis=-1, eps=1e-05):
    m = jnp.mean(x, axis=axis, keepdims=True)
    v = jnp.var(x, axis=axis, keepdims=True)
    return (x - m) / jnp.sqrt(v + eps)

def _scatter_add(tgt, idx, src, axis=0):
    return tgt.at[idx].add(src)

def _segment_sum(src, seg, n):
    return jax.ops.segment_sum(src, seg, n)

class _Rng:

    def __init__(self, key):
        self._k = key

    def _next(self):
        self._k, sub = jax.random.split(self._k)
        return sub

    def normal(self, shape):
        return jax.random.normal(self._next(), shape, dtype=jnp.bfloat16)

    def randint(self, lo, hi, shape):
        return jax.random.randint(self._next(), shape, lo, hi, dtype=jnp.int32)

    def uniform(self, shape, lo=0.0, hi=1.0):
        return jax.random.uniform(self._next(), shape, jnp.bfloat16, lo, hi)

    def permutation(self, n):
        return jax.random.permutation(self._next(), n)
kernel_name = 'adaLN_cond__sliding_local_dilated__glu_gated_swiglu__prompt'

def setup_inputs():
    _rng = _Rng(jax.random.key(int.from_bytes(__import__("os").urandom(4), "little")))
    _w = lambda a: (lambda t: t.astype(jnp.bfloat16) if jnp.issubdtype(t.dtype, jnp.floating) else t)(jnp.asarray(a))

    def _A_setup():
        B, S, D = (1, 2048, 1024)
        return {'x': _w((lambda *s: _rng.normal(s) * 0.05)(B, S, D)), 'wqkv': _w((lambda *s: _rng.normal(s) * 0.05)(D, 3 * D)), 'wo': _w((lambda *s: _rng.normal(s) * 0.05)(D, D))}
    _A_in = _A_setup()

    def _B_setup():
        B, S, D, F = (1, 2048, 1024, 3584)
        return {'x': _w((lambda *s: _rng.normal(s) * 0.05)(B, S, D)), 'w1': _w((lambda *s: _rng.normal(s) * 0.05)(D, F) * (2.0 / D) ** 0.5), 'w3': _w((lambda *s: _rng.normal(s) * 0.05)(D, F) * (2.0 / D) ** 0.5), 'w2': _w((lambda *s: _rng.normal(s) * 0.05)(F, D) * (2.0 / F) ** 0.5)}
    _B_in = _B_setup()
    return {'A_x': _A_in['x'], 'A_wqkv': _A_in['wqkv'], 'A_wo': _A_in['wo'], 'B_x': _B_in['x'], 'B_w1': _B_in['w1'], 'B_w3': _B_in['w3'], 'B_w2': _B_in['w2'], 'c': _w((lambda *s: _rng.normal(s) * 0.05)(1, 1024)), 'w_mod': _w((lambda *s: _rng.normal(s) * 0.05)(1024, 6 * 1024) * 1024 ** (-0.5))}

def reference(A_x, A_wqkv, A_wo, B_x, B_w1, B_w3, B_w2, c, w_mod):

    def _A_ref(x, wqkv, wo):
        B, S, D = x.shape
        H = 32
        Dh = D // H
        W, dil = (8, 2)
        qkv = (lambda x, *d: x.transpose(*d))((x @ wqkv).reshape(B, S, 3, H, Dh), 2, 0, 3, 1, 4)
        q, k, v = (qkv[0], qkv[1], qkv[2])
        scale = Dh ** (-0.5)
        pos = jnp.arange(S)
        off = jnp.arange(W) * dil
        idx = pos[:, None] - off[None, :]
        mask = idx >= 0
        idx_c = jnp.where(mask, idx, 0).reshape(-1)
        kg = k[:, :, idx_c, :].reshape(B, H, S, W, Dh)
        vg = v[:, :, idx_c, :].reshape(B, H, S, W, Dh)
        logits = jnp.einsum('bhsd,bhswd->bhsw', q, kg) * scale
        logits = jnp.where(mask[None, None, :, :], logits, -1000000000.0)
        attn = _softmax(logits, axis=-1)
        o = jnp.einsum('bhsw,bhswd->bhsd', attn, vg)
        return (lambda x, *d: x.transpose(*d))(o, 0, 2, 1, 3).reshape(B, S, D) @ wo

    def _B_ref(x, w1, w3, w2):
        gate = jnp.einsum('bsd,df->bsf', x, w1)
        up = jnp.einsum('bsd,df->bsf', x, w3)
        h = _silu(gate) * up
        out = jnp.einsum('bsf,fd->bsd', h, w2)
        return out
    x = A_x
    mod = (_silu(c) @ w_mod).reshape(c.shape[0], 6, 1, -1)
    sa, ca, ga, sb, cb, gb = (mod[:, 0].copy(), mod[:, 1].copy(), mod[:, 2].copy(), mod[:, 3].copy(), mod[:, 4].copy(), mod[:, 5].copy())
    h = _layernorm(x, axis=-1) * (1 + ca) + sa
    x = x + ga * _A_ref(h, A_wqkv, A_wo)
    h = _layernorm(x, axis=-1) * (1 + cb) + sb
    x = x + gb * _B_ref(h, B_w1, B_w3, B_w2)
    return x
```

```python
import jax
import jax.numpy as jnp
from jax import lax
import jax.experimental.pallas as pl
import jax.experimental.pallas.tpu as pltpu

S, D, F = 2048, 1024, 3584
H, DH, WIN, DIL = 32, 32, 8, 2
HALO = 16
T, HM = 256, 128
NT = S // T
NFT = F // 128
AB = 16
LB = 32
LOG2E = 1.4426950408889634
NEG = -1e9 * LOG2E
BF16, F32, U32, I32 = jnp.bfloat16, jnp.float32, jnp.uint32, jnp.int32


def _nt(a, b):
    return lax.dot_general(a, b, (((1,), (1,)), ((), ())), preferred_element_type=F32)


def _nn(a, b):
    return jnp.dot(a, b, preferred_element_type=F32)


def _bf(x):
    return pltpu.bitcast(x, BF16)


def _recip(d):
    y = pltpu.bitcast(0x7EF311C7 - pltpu.bitcast(d, I32), F32)
    for _ in range(3):
        y = y * (2.0 - d * y)
    return y


def _rsqrt(d):
    y = pltpu.bitcast(0x5F375A86 - (pltpu.bitcast(d, I32) >> 1), F32)
    hd = 0.5 * d
    for _ in range(4):
        y = y * (1.5 - hd * y * y)
    return y


def _layernorm(x):
    m = jnp.mean(x, axis=-1, keepdims=True)
    d = x - m
    v = jnp.mean(d * d, axis=-1, keepdims=True)
    return d * _rsqrt(v + 1e-5)


def _a_ops(a11, a12, a21, a22):
    return [a11 + a22, a21 + a22, a11, a22, a11 + a12, a21 - a11, a12 - a22]


def _b_ops(b11, b12, b21, b22):
    return [b11 + b22, b11, b12 - b22, b21 - b11, b22, b11 + b12, b21 + b22]


def _c_blocks(m):
    return (m[0] + m[3] - m[4] + m[6], m[2] + m[4], m[1] + m[3], m[0] - m[1] + m[2] + m[5])


def _kernel(zero_s, x_hbm, wqkv_hbm, wo_hbm, w1_hbm, w3_hbm, w2_hbm, c_hbm, wmod_hbm, out_hbm,
            mod_v, so_b, sa_b, tq_b, to_b, q_v, k_v, v_v, x_v, act_b, tu_b, td_b, c_v, wm_v, wraw_v, t0_b, woraw_b, sem):
    mo = pl.multiple_of
    t0_v, tq_v, woraw_v, to_v = (r.bitcast(U32) for r in (t0_b, tq_b, woraw_b, to_b))
    tu_v, td_v, sa_v, so_v, act_v = (r.bitcast(U32) for r in (tu_b, td_b, sa_b, so_b, act_b))
    r_v = q_v
    x1_v = k_v

    names = {}

    def sidx(name):
        if name not in names:
            names[name] = len(names)
        return sem.at[names[name]]

    def cp(src, dst, name):
        return pltpu.make_async_copy(src, dst, sidx(name))

    def x_cp(i):
        return cp(x_hbm.at[i * T:(i + 1) * T, :], x_v.at[i * T:(i + 1) * T, :], ("x", i))

    def wm_cp(j):
        return cp(wmod_hbm.at[:, j * 512:(j + 1) * 512], wm_v.at[j], ("wm", j))

    def w_cp(p):
        return cp(wqkv_hbm.at[:, p * D:(p + 1) * D], wraw_v.at[p], ("w", p))

    def wo_cp():
        return cp(woraw_b, woraw_b, "wo")

    def up_grp_wait(g):
        blk = tu_b.at[pl.ds(g * 6, 6), 1:5]
        return pltpu.make_async_copy(blk, blk, sem.at[40 + g])

    def dn_grp(j):
        blk = td_b.at[1:5, j, 0:NFT // 2]
        return cp(blk, blk, ("w2", j))

    c_cp = cp(c_hbm, c_v, "c")
    c_cp.start()
    for j in range(4):
        wm_cp(j).start()
    x_cp(0).start()
    for p in range(3):
        w_cp(p).start()
    x_cp(1).start()
    x_cp(2).start()
    for j in range(8):
        pltpu.make_async_copy(wo_hbm.at[:, j * 128:(j + 1) * 128], woraw_b.at[j], sidx("wo")).start()
    wm_cp(4).start()
    wm_cp(5).start()
    for i in range(3, NT):
        x_cp(i).start()

    def start_up(g):
        for nt in range(6 * g, 6 * g + 6):
            cs = slice(min(nt, NFT - 1) * 128, (min(nt, NFT - 1) + 1) * 128)
            sm_ = sem.at[40 + g]
            pltpu.make_async_copy(w1_hbm.at[0:512, cs], tu_b.at[nt, 1], sm_).start()
            pltpu.make_async_copy(w3_hbm.at[0:512, cs], tu_b.at[nt, 2], sm_).start()
            pltpu.make_async_copy(w1_hbm.at[512:1024, cs], tu_b.at[nt, 3], sm_).start()
            pltpu.make_async_copy(w3_hbm.at[512:1024, cs], tu_b.at[nt, 4], sm_).start()

    def start_dn(j):
        for kh in range(2):
            for nh in range(2):
                c0 = nh * 512 + j * 128
                pltpu.make_async_copy(w2_hbm.at[:, kh, :, c0:c0 + 128], td_b.at[1 + 2 * kh + nh, j, 0:NFT // 2],
                                      sidx(("w2", j))).start()

    def mod_chunk(j, sc16, wait=True):
        if wait:
            wm_cp(j).wait()
        r = _nn(sc16, wm_v[j])[0:8]
        if j // 2 in (1, 4):
            r = r + 1.0
        mod_v[:, j * 512:(j + 1) * 512] = r
        return r

    def silu_c():
        cc = c_v[...].astype(F32)
        return jnp.broadcast_to((cc * jax.nn.sigmoid(cc)).astype(BF16), (16, D))

    def modp(i):
        return mod_v[0:1, i * D:(i + 1) * D]

    def prep_w(p, wait=True):
        if wait:
            w_cp(p).wait()
        for kt in range(8):
            t0_b[kt] = wraw_v[p, kt * 128:(kt + 1) * 128, :].T
        for jp in range(4):
            for kt in range(4):
                for g in range(2):
                    def rows(j, k):
                        return _bf(t0_v[k, pl.ds(2 * j + g, 32, stride=16), :]).astype(F32)
                    ops = _b_ops(rows(jp, kt), rows(jp + 4, kt), rows(jp, kt + 4), rows(jp + 4, kt + 4))
                    for i in range(7):
                        tq_b[p * 4 + jp, i, kt, g * 64:(g + 1) * 64, :] = ops[i].astype(BF16)

    def prep_wo():
        for nt in range(4):
            for dp in range(8):
                def rows(j, d):
                    return _bf(woraw_v[j, pl.ds(d, 32, stride=16), :]).astype(F32)
                ops = _b_ops(rows(nt, dp), rows(nt + 4, dp), rows(nt, dp + 8), rows(nt + 4, dp + 8))
                for i in range(7):
                    to_b[i, nt, dp * 64:(dp + 1) * 64, :] = ops[i].astype(BF16)

    def after(tok, val):
        if tok is None:
            return val
        t = tok[0:val.shape[0], :]
        return jnp.where(never[0:val.shape[0]], t if t.dtype == val.dtype else pltpu.bitcast(t, val.dtype), val)

    def weight_sums(raw, tok):
        raw = [after(tok, raw[0]), raw[1], raw[2], after(tok, raw[3])]
        b11, b12, b21, b22 = (_bf(r).astype(F32) for r in raw)
        return ((0, b11 + b22), (2, b12 - b22), (3, b21 - b11), (5, b11 + b12), (6, b21 + b22))

    def prep_up(nt, toks):
        for n, rb in enumerate(range(0, 512, 128)):
            sl = slice(rb // 2, (rb + 128) // 2)
            for s, val in weight_sums([tu_v[nt, q, sl, :] for q in (1, 2, 3, 4)], toks[n]):
                tu_b[nt, s, rb:rb + 128, :] = val.astype(BF16)

    def prep_dn(cpi, toks):
        for j in range(4):
            for s, val in weight_sums([td_v[q, j, cpi] for q in (1, 2, 3, 4)], toks[j]):
                td_b[s, j, cpi] = val.astype(BF16)

    def ln_tile(load, mi, slot):
        for b in range(0, HM, LB):
            hs = [_layernorm(load(ro + b)) * modp(mi + 1) + modp(mi) for ro in (0, HM)]
            ops = _a_ops(hs[0][:, :512], hs[0][:, 512:], hs[1][:, :512], hs[1][:, 512:])
            for i in range(7):
                for kt in range(4):
                    sa_b[slot, i, kt, b:b + LB, :] = ops[i][:, kt * 128:(kt + 1) * 128].astype(BF16)

    def ln1(r0, slot):
        ln_tile(lambda r: x_v[pl.ds(mo(r0 + r, LB), LB), :].astype(F32), 0, slot)

    def ln2(r0, slot, toks=None):
        def load(r):
            cols = [x1_v[j, pl.ds(mo(HALO + r0 + r, 16), LB), :] for j in range(8)]
            if toks is not None:
                cols[0] = after(toks[(r % HM) // LB * 2 + r // HM], cols[0])
            return jnp.concatenate(cols, axis=1)
        ln_tile(load, 3, slot)

    def qkv(r0, slot, prs=range(12)):
        toks = []
        for pr in prs:
            m = []
            for i in range(7):
                acc = None
                for kt in range(4):
                    t = _nt(_bf(sa_v[slot, i, kt]), _bf(tq_v[pr, i, kt]))
                    acc = t if acc is None else acc + t
                m.append(acc)
            toks += m
            c = _c_blocks(m)
            p, jp = pr // 4, pr % 4
            dst, off = ((q_v, 0), (k_v, HALO), (v_v, HALO))[p]
            for hf in range(2):
                for sd in range(2):
                    val = c[hf * 2 + sd]
                    if p == 0:
                        val = val * (LOG2E * DH ** -0.5)
                    dst[jp + 4 * sd, pl.ds(mo(off + r0 + hf * HM, 16), HM), :] = val
        return toks

    never = lax.broadcasted_iota(I32, (128, 128), 1) < zero_s[0]
    lane = lax.broadcasted_iota(I32, (AB, 128), 1)
    even = (lane & 1) == 0
    rowi = lax.broadcasted_iota(I32, (AB, 128), 0)

    def qkred(r0, first=False):
        for b in range(0, T, AB):
            rb = r0 + b
            qs = [q_v[jp, pl.ds(rb, AB), :] for jp in range(8)]
            rrs = []
            for w in range(WIN):
                rr = None
                for jp in range(8):
                    t = qs[jp] * k_v[jp, pl.ds(rb + (HALO - DIL * w), AB), :]
                    rr = t if rr is None else rr + t
                rrs.append(rr)
            s1s = [rr + pltpu.roll(rr, 64, 1) for rr in rrs]
            for w, s1 in enumerate(s1s):
                l = s1 + jnp.where(even, pltpu.roll(s1, 127, 1), pltpu.roll(s1, 1, 1))
                if first and b < DIL * w:
                    l = jnp.where(rowi + b >= DIL * w, l, NEG)
                r_v[w, pl.ds(rb, AB), :] = l

    def sm(r0):
        for b in range(0, T, AB):
            ls = [r_v[w, pl.ds(r0 + b, AB), :] for w in range(WIN)]
            m = ls[0]
            for w in range(1, WIN):
                m = jnp.maximum(m, ls[w])
            for w in range(WIN):
                r_v[w, pl.ds(r0 + b, AB), :] = jnp.exp2(ls[w] - m)

    def pv_blk(rb):
        es = [r_v[w, pl.ds(rb, AB), :] for w in range(WIN)]
        den = es[0]
        for w in range(1, WIN):
            den = den + es[w]
        inv = _recip(den)
        out = []
        for jp in range(8):
            oo = None
            for w in range(WIN):
                t = es[w] * v_v[jp, pl.ds(rb + (HALO - DIL * w), AB), :]
                oo = t if oo is None else oo + t
            out.append(oo * inv)
        return out

    def pv(r0):
        for b in range(0, HM, AB):
            ot, ob = pv_blk(r0 + b), pv_blk(r0 + HM + b)
            ops = _a_ops(jnp.concatenate(ot[:4], axis=1), jnp.concatenate(ot[4:], axis=1),
                         jnp.concatenate(ob[:4], axis=1), jnp.concatenate(ob[4:], axis=1))
            for i in range(7):
                for kt in range(4):
                    so_b[i, kt, b:b + AB, :] = ops[i][:, kt * 128:(kt + 1) * 128].astype(BF16)

    def wo(r0):
        for nt in range(4):
            m = []
            for i in range(7):
                acc = None
                for kt in range(4):
                    t = _nn(_bf(so_v[i, kt]), _bf(to_v[i, nt, kt * 64:(kt + 1) * 64, :]))
                    acc = t if acc is None else acc + t
                m.append(acc)
            c = _c_blocks(m)
            for hf in range(2):
                for sd in range(2):
                    j = nt + 4 * sd
                    cs = slice(j * 128, (j + 1) * 128)
                    xx = x_v[pl.ds(mo(r0 + hf * HM, HM), HM), cs].astype(F32)
                    ga = mod_v[0:1, 2 * D + j * 128:2 * D + (j + 1) * 128]
                    x1_v[j, pl.ds(mo(HALO + r0 + hf * HM, 16), HM), :] = xx + ga * c[hf * 2 + sd]

    def block(fn):
        pl.when(zero_s[0] == 0)(fn)

    dz = zero_s[0]
    start_up(0)
    c_cp.wait()
    sc16 = silu_c()
    for j in range(4):
        mod_chunk(j, sc16)
    x_cp(0).wait()
    ln1(0, 0)
    k_v[:, 0:HALO, :] = jnp.zeros((8, HALO, 128), F32)
    prep_w(0)
    w_cp(1).wait()
    qkv(0, 0, range(0, 4))
    prep_w(1, wait=False)
    w_cp(2).wait()
    qkv(0, 0, range(4, 8))
    prep_w(2, wait=False)

    def tile(k):
        i = k + (zero_s[0] + 7) % 7
        return i, mo(i * T, T)

    @block
    def _():
        start_up(1)
        x_cp(1).wait()
        i, r0 = tile(0)
        qkv(r0, i, range(8, 12))
        ln1(r0 + T, i + 1)

    @block
    def _():
        x_cp(2).wait()
        wo_cp().wait()
        i, r0 = tile(1)
        v_v[:, 0:HALO, :] = jnp.broadcast_to(v_v[:, HALO:HALO + 1, :], (8, HALO, 128))
        qkv(r0, i)
        qkred(r0 - T, first=True)
        ln1(r0 + T, i + 1)
        prep_wo()

    @block
    def _():
        start_up(2)
        x_cp(3).wait()
        wm_cp(4).wait()
        wm_cp(5).wait()
        i, r0 = tile(2)
        sc = silu_c()
        mod_chunk(4, sc, wait=False)
        mod_chunk(5, sc, wait=False)
        qkv(r0, i)
        sm(r0 - 2 * T)
        qkred(r0 - T)
        ln1(r0 + T, i + 1)

    for i in range(4, NT):
        x_cp(i).wait()

    def mid_body(it, carry):
        @pl.when(it == 0)
        def _():
            start_up(3)
            for j in range(4):
                start_dn(j)

        @pl.when(it == 1)
        def _():
            start_up(4)
            for j in range(6, 12):
                wm_cp(j).start()

        up_grp_wait(it).wait()

        @pl.when(it == 2)
        def _():
            for j in range(4):
                dn_grp(j).wait()

        i = 3 + it % 5
        r0 = mo(i * T, T)
        toks = qkv(r0, i)
        pv(r0 - 3 * T)
        wo(r0 - 3 * T)
        sm(r0 - 2 * T)
        qkred(r0 - T)
        ln1(mo(jnp.minimum(r0 + T, S - T), T), i + 1)
        pieces = 6 * 4 + 5 * 4
        tk = [toks[8 + (len(toks) - 9) * n // pieces] for n in range(pieces)]
        for n in range(6):
            prep_up((i - 3) * 6 + n, tk[4 * n:4 * n + 4])
        for n in range(5):
            prep_dn(jnp.where(i >= 5, 5 * (i - 5) + n, NFT // 2), tk[24 + 4 * n:28 + 4 * n])
        return carry

    lax.fori_loop(0, 5, mid_body, 0)

    @block
    def _():
        for j in range(6, 12):
            wm_cp(j).wait()
        i, r0 = tile(8)
        sc = silu_c()
        for j in range(6, 12):
            mod_chunk(j, sc, wait=False)
        pv(r0 - 3 * T)
        wo(r0 - 3 * T)
        sm(r0 - 2 * T)
        qkred(r0 - T)

    @block
    def _():
        i, r0 = tile(9)
        pv(r0 - 3 * T)
        wo(r0 - 3 * T)
        sm(r0 - 2 * T)
        ln2(r0 - 9 * T, i - 9)

    @block
    def _():
        i, r0 = tile(10)
        pv(r0 - 3 * T)
        wo(r0 - 3 * T)

    def out_cp(r0, r):
        return pltpu.make_async_copy(x_v.at[pl.ds(r0, T), :], out_hbm.at[pl.ds(r0, T), :], sem.at[48 + r])

    def ffn_body(it, carry):
        r = it % NT
        r0 = mo(r * T, T)
        toks = []
        for cpair in range(NFT // 2):
            acts = []
            for nt in (2 * cpair, 2 * cpair + 1):
                m = []
                for i in range(7):
                    acc = None
                    for kt in range(4):
                        t = _nn(_bf(sa_v[r, i, kt]), _bf(tu_v[nt, i, kt * 64:(kt + 1) * 64, :]))
                        acc = t if acc is None else acc + t
                    m.append(acc)
                toks += m
                gt, ut, gb, ub = _c_blocks(m)
                acts.append((gt * jax.nn.sigmoid(gt) * ut, gb * jax.nn.sigmoid(gb) * ub))
            (a11, a21), (a12, a22) = acts
            ops = _a_ops(a11, a12, a21, a22)
            for i in range(7):
                act_b[i, cpair] = ops[i].astype(BF16)
        ln2(mo(jnp.minimum(r0 + T, S - T), T), r + 1,
            [toks[int(len(toks) * (0.05 + 0.55 * n / 8))] for n in range(8)])
        for j in range(4):
            m = []
            for i in range(7):
                acc = None
                for cpair in range(NFT // 2):
                    t = _nn(_bf(act_v[i, cpair]), _bf(td_v[i, j, cpair]))
                    acc = t if acc is None else acc + t
                m.append(acc)
            c = _c_blocks(m)
            for hf in range(2):
                for sd in range(2):
                    jj = j + 4 * sd
                    cs = slice(jj * 128, (jj + 1) * 128)
                    gb = mod_v[0:1, 5 * D + jj * 128:5 * D + (jj + 1) * 128]
                    res = x1_v[jj, pl.ds(mo(HALO + r0 + hf * HM, 16), HM), :] + gb * c[hf * 2 + sd]
                    x_v[pl.ds(mo(r0 + hf * HM, HM), HM), cs] = res.astype(BF16)
        out_cp(r0, r).start()
        return carry

    lax.fori_loop(0, NT, ffn_body, 0)
    for r in range(NT):
        out_cp(r * T, r).wait()


@jax.jit
def pallas_adaLN_cond__sliding_local_dilated__glu_gated_swiglu__prompt_kernel(
    A_x, A_wqkv, A_wo, B_x, B_w1, B_w3, B_w2, c, w_mod,
):
    del B_x
    any_spec = pl.BlockSpec(memory_space=pl.ANY)
    scratch = [
        pltpu.VMEM((8, 6 * D), F32),
        pltpu.VMEM((7, 4, HM, 128), BF16),
        pltpu.VMEM((NT + 1, 7, 4, HM, 128), BF16),
        pltpu.VMEM((12, 7, 4, 128, 128), BF16),
        pltpu.VMEM((7, 4, 512, 128), BF16),
        pltpu.VMEM((8, S, 128), F32),
        pltpu.VMEM((8, S + HALO, 128), F32),
        pltpu.VMEM((8, S + HALO, 128), F32),
        pltpu.VMEM((S, D), BF16),
        pltpu.VMEM((7, NFT // 2, HM, 128), BF16),
        pltpu.VMEM((NFT + 2, 7, 512, 128), BF16),
        pltpu.VMEM((7, 4, NFT // 2 + 1, 128, 128), BF16),
        pltpu.VMEM((1, D), BF16),
        pltpu.VMEM((12, D, 512), BF16),
        pltpu.VMEM((3, D, D), BF16),
        pltpu.VMEM((8, D, 128), BF16),
        pltpu.VMEM((8, D, 128), BF16),
        pltpu.SemaphoreType.DMA((64,)),
    ]
    out = pl.pallas_call(
        _kernel,
        out_shape=jax.ShapeDtypeStruct((S, D), BF16),
        in_specs=[pl.BlockSpec(memory_space=pltpu.SMEM)] + [any_spec] * 8,
        out_specs=any_spec,
        scratch_shapes=scratch,
        compiler_params=pltpu.CompilerParams(vmem_limit_bytes=126 * 1024 * 1024),
    )(jnp.zeros((1,), I32), A_x.reshape(S, D), A_wqkv, A_wo, B_w1, B_w3, B_w2.reshape(NFT // 2, 2, 128, D), c, w_mod)
    return out.reshape(1, S, D)
```

```python
import jax
import jax.numpy as jnp
from jax import lax
import jax.experimental.pallas as pl
import jax.experimental.pallas.tpu as pltpu

S, D, F = 2048, 1024, 3584
H, DH, WIN, DIL = 32, 32, 8, 2
HALO = 16
T, HM = 256, 128
NT = S // T
NFT = F // 128
AB = 16
LB = 32
LOG2E = 1.4426950408889634
NEG = -1e9 * LOG2E
BF16, F32, U32, I32 = jnp.bfloat16, jnp.float32, jnp.uint32, jnp.int32


def _nt(a, b):
    return lax.dot_general(a, b, (((1,), (1,)), ((), ())), preferred_element_type=F32)


def _nn(a, b):
    return jnp.dot(a, b, preferred_element_type=F32)


def _bf(x):
    return pltpu.bitcast(x, BF16)


def _recip(d):
    y = pltpu.bitcast(0x7EF311C7 - pltpu.bitcast(d, I32), F32)
    for _ in range(3):
        y = y * (2.0 - d * y)
    return y


def _rsqrt(d):
    y = pltpu.bitcast(0x5F375A86 - (pltpu.bitcast(d, I32) >> 1), F32)
    hd = 0.5 * d
    for _ in range(4):
        y = y * (1.5 - hd * y * y)
    return y


def _layernorm(x):
    m = jnp.mean(x, axis=-1, keepdims=True)
    d = x - m
    v = jnp.mean(d * d, axis=-1, keepdims=True)
    return d * _rsqrt(v + 1e-5)


def _a_ops(a11, a12, a21, a22):
    return [a11 + a22, a21 + a22, a11, a22, a11 + a12, a21 - a11, a12 - a22]


def _b_ops(b11, b12, b21, b22):
    return [b11 + b22, b11, b12 - b22, b21 - b11, b22, b11 + b12, b21 + b22]


def _c_blocks(m):
    return (m[0] + m[3] - m[4] + m[6], m[2] + m[4], m[1] + m[3], m[0] - m[1] + m[2] + m[5])


def _kernel(zero_s, x_hbm, wqkv_hbm, wo_hbm, w1_hbm, w3_hbm, w2_hbm, c_hbm, wmod_hbm, out_hbm,
            mod_v, so_b, sa_b, tq_b, to_b, q_v, k_v, v_v, x_v, act_b, tu_b, td_b, c_v, wm_v, wraw_v, t0_b, woraw_b, sem):
    mo = pl.multiple_of
    t0_v, tq_v, woraw_v, to_v = (r.bitcast(U32) for r in (t0_b, tq_b, woraw_b, to_b))
    tu_v, td_v, sa_v, so_v, act_v = (r.bitcast(U32) for r in (tu_b, td_b, sa_b, so_b, act_b))
    r_v = q_v
    x1_v = k_v

    names = {}

    def sidx(name):
        if name not in names:
            names[name] = len(names)
        return sem.at[names[name]]

    def cp(src, dst, name):
        return pltpu.make_async_copy(src, dst, sidx(name))

    def x_cp(i):
        return cp(x_hbm.at[i * T:(i + 1) * T, :], x_v.at[i * T:(i + 1) * T, :], ("x", i))

    def wm_cp(j):
        return cp(wmod_hbm.at[:, j * 512:(j + 1) * 512], wm_v.at[j], ("wm", j))

    def w_cp(p):
        return cp(wqkv_hbm.at[:, p * D:(p + 1) * D], wraw_v.at[p], ("w", p))

    def wo_cp():
        return cp(woraw_b, woraw_b, "wo")

    def up_grp_wait(g):
        blk = tu_b.at[pl.ds(g * 6, 6), 1:5]
        return pltpu.make_async_copy(blk, blk, sem.at[40 + g])

    def dn_grp(j):
        blk = td_b.at[1:5, j, 0:NFT // 2]
        return cp(blk, blk, ("w2", j))

    c_cp = cp(c_hbm, c_v, "c")
    c_cp.start()
    for j in range(4):
        wm_cp(j).start()
    x_cp(0).start()
    for p in range(3):
        w_cp(p).start()
    x_cp(1).start()
    x_cp(2).start()
    for j in range(8):
        pltpu.make_async_copy(wo_hbm.at[:, j * 128:(j + 1) * 128], woraw_b.at[j], sidx("wo")).start()
    wm_cp(4).start()
    wm_cp(5).start()
    for i in range(3, NT):
        x_cp(i).start()

    def start_up(g):
        for nt in range(6 * g, 6 * g + 6):
            cs = slice(min(nt, NFT - 1) * 128, (min(nt, NFT - 1) + 1) * 128)
            sm_ = sem.at[40 + g]
            pltpu.make_async_copy(w1_hbm.at[0:512, cs], tu_b.at[nt, 1], sm_).start()
            pltpu.make_async_copy(w3_hbm.at[0:512, cs], tu_b.at[nt, 2], sm_).start()
            pltpu.make_async_copy(w1_hbm.at[512:1024, cs], tu_b.at[nt, 3], sm_).start()
            pltpu.make_async_copy(w3_hbm.at[512:1024, cs], tu_b.at[nt, 4], sm_).start()

    def start_dn(j):
        for kh in range(2):
            for nh in range(2):
                c0 = nh * 512 + j * 128
                pltpu.make_async_copy(w2_hbm.at[:, kh, :, c0:c0 + 128], td_b.at[1 + 2 * kh + nh, j, 0:NFT // 2],
                                      sidx(("w2", j))).start()

    def mod_chunk(j, sc16, wait=True):
        if wait:
            wm_cp(j).wait()
        r = _nn(sc16, wm_v[j])[0:8]
        if j // 2 in (1, 4):
            r = r + 1.0
        mod_v[:, j * 512:(j + 1) * 512] = r
        return r

    def silu_c():
        cc = c_v[...].astype(F32)
        return jnp.broadcast_to((cc * jax.nn.sigmoid(cc)).astype(BF16), (16, D))

    def modp(i):
        return mod_v[0:1, i * D:(i + 1) * D]

    def prep_w(p, wait=True):
        if wait:
            w_cp(p).wait()
        for kt in range(8):
            t0_b[kt] = wraw_v[p, kt * 128:(kt + 1) * 128, :].T
        for jp in range(4):
            for kt in range(4):
                for g in range(2):
                    def rows(j, k):
                        return _bf(t0_v[k, pl.ds(2 * j + g, 32, stride=16), :]).astype(F32)
                    ops = _b_ops(rows(jp, kt), rows(jp + 4, kt), rows(jp, kt + 4), rows(jp + 4, kt + 4))
                    for i in range(7):
                        tq_b[p * 4 + jp, i, kt, g * 64:(g + 1) * 64, :] = ops[i].astype(BF16)

    def prep_wo():
        for nt in range(4):
            for dp in range(8):
                def rows(j, d):
                    return _bf(woraw_v[j, pl.ds(d, 32, stride=16), :]).astype(F32)
                ops = _b_ops(rows(nt, dp), rows(nt + 4, dp), rows(nt, dp + 8), rows(nt + 4, dp + 8))
                for i in range(7):
                    to_b[i, nt, dp * 64:(dp + 1) * 64, :] = ops[i].astype(BF16)

    def after(tok, val):
        if tok is None:
            return val
        t = tok[0:val.shape[0], :]
        return jnp.where(never[0:val.shape[0]], t if t.dtype == val.dtype else pltpu.bitcast(t, val.dtype), val)

    def weight_sums(raw, tok):
        raw = [after(tok, raw[0]), raw[1], raw[2], after(tok, raw[3])]
        b11, b12, b21, b22 = (_bf(r).astype(F32) for r in raw)
        return ((0, b11 + b22), (2, b12 - b22), (3, b21 - b11), (5, b11 + b12), (6, b21 + b22))

    def prep_up(nt, toks):
        for n, rb in enumerate(range(0, 512, 128)):
            sl = slice(rb // 2, (rb + 128) // 2)
            for s, val in weight_sums([tu_v[nt, q, sl, :] for q in (1, 2, 3, 4)], toks[n]):
                tu_b[nt, s, rb:rb + 128, :] = val.astype(BF16)

    def prep_dn(cpi, toks):
        for j in range(4):
            for s, val in weight_sums([td_v[q, j, cpi] for q in (1, 2, 3, 4)], toks[j]):
                td_b[s, j, cpi] = val.astype(BF16)

    def ln_tile(load, mi, slot):
        for b in range(0, HM, LB):
            hs = [_layernorm(load(ro + b)) * modp(mi + 1) + modp(mi) for ro in (0, HM)]
            ops = _a_ops(hs[0][:, :512], hs[0][:, 512:], hs[1][:, :512], hs[1][:, 512:])
            for i in range(7):
                for kt in range(4):
                    sa_b[slot, i, kt, b:b + LB, :] = ops[i][:, kt * 128:(kt + 1) * 128].astype(BF16)

    def ln1(r0, slot):
        ln_tile(lambda r: x_v[pl.ds(mo(r0 + r, LB), LB), :].astype(F32), 0, slot)

    def ln2(r0, slot, toks=None):
        def load(r):
            cols = [x1_v[j, pl.ds(mo(HALO + r0 + r, 16), LB), :] for j in range(8)]
            if toks is not None:
                cols[0] = after(toks[(r % HM) // LB * 2 + r // HM], cols[0])
            return jnp.concatenate(cols, axis=1)
        ln_tile(load, 3, slot)

    def qkv(r0, slot, prs=range(12)):
        toks = []
        for pr in prs:
            m = []
            for i in range(7):
                acc = None
                for kt in range(4):
                    t = _nt(_bf(sa_v[slot, i, kt]), _bf(tq_v[pr, i, kt]))
                    acc = t if acc is None else acc + t
                m.append(acc)
            toks += m
            c = _c_blocks(m)
            p, jp = pr // 4, pr % 4
            dst, off = ((q_v, 0), (k_v, HALO), (v_v, HALO))[p]
            for hf in range(2):
                for sd in range(2):
                    val = c[hf * 2 + sd]
                    if p == 0:
                        val = val * (LOG2E * DH ** -0.5)
                    dst[jp + 4 * sd, pl.ds(mo(off + r0 + hf * HM, 16), HM), :] = val
        return toks

    never = lax.broadcasted_iota(I32, (128, 128), 1) < zero_s[0]
    lane = lax.broadcasted_iota(I32, (AB, 128), 1)
    even = (lane & 1) == 0
    rowi = lax.broadcasted_iota(I32, (AB, 128), 0)

    def qkred(r0, first=False):
        for b in range(0, T, AB):
            rb = r0 + b
            qs = [q_v[jp, pl.ds(rb, AB), :] for jp in range(8)]
            rrs = []
            for w in range(WIN):
                rr = None
                for jp in range(8):
                    t = qs[jp] * k_v[jp, pl.ds(rb + (HALO - DIL * w), AB), :]
                    rr = t if rr is None else rr + t
                rrs.append(rr)
            s1s = [rr + pltpu.roll(rr, 64, 1) for rr in rrs]
            for w, s1 in enumerate(s1s):
                l = s1 + jnp.where(even, pltpu.roll(s1, 127, 1), pltpu.roll(s1, 1, 1))
                if first and b < DIL * w:
                    l = jnp.where(rowi + b >= DIL * w, l, NEG)
                r_v[w, pl.ds(rb, AB), :] = l

    def sm(r0):
        for b in range(0, T, AB):
            ls = [r_v[w, pl.ds(r0 + b, AB), :] for w in range(WIN)]
            m = ls[0]
            for w in range(1, WIN):
                m = jnp.maximum(m, ls[w])
            for w in range(WIN):
                r_v[w, pl.ds(r0 + b, AB), :] = jnp.exp2(ls[w] - m)

    def pv_blk(rb):
        es = [r_v[w, pl.ds(rb, AB), :] for w in range(WIN)]
        den = es[0]
        for w in range(1, WIN):
            den = den + es[w]
        inv = _recip(den)
        out = []
        for jp in range(8):
            oo = None
            for w in range(WIN):
                t = es[w] * v_v[jp, pl.ds(rb + (HALO - DIL * w), AB), :]
                oo = t if oo is None else oo + t
            out.append(oo * inv)
        return out

    def pv(r0):
        for b in range(0, HM, AB):
            ot, ob = pv_blk(r0 + b), pv_blk(r0 + HM + b)
            ops = _a_ops(jnp.concatenate(ot[:4], axis=1), jnp.concatenate(ot[4:], axis=1),
                         jnp.concatenate(ob[:4], axis=1), jnp.concatenate(ob[4:], axis=1))
            for i in range(7):
                for kt in range(4):
                    so_b[i, kt, b:b + AB, :] = ops[i][:, kt * 128:(kt + 1) * 128].astype(BF16)

    def wo(r0):
        for nt in range(4):
            m = []
            for i in range(7):
                acc = None
                for kt in range(4):
                    t = _nn(_bf(so_v[i, kt]), _bf(to_v[i, nt, kt * 64:(kt + 1) * 64, :]))
                    acc = t if acc is None else acc + t
                m.append(acc)
            c = _c_blocks(m)
            for hf in range(2):
                for sd in range(2):
                    j = nt + 4 * sd
                    cs = slice(j * 128, (j + 1) * 128)
                    xx = x_v[pl.ds(mo(r0 + hf * HM, HM), HM), cs].astype(F32)
                    ga = mod_v[0:1, 2 * D + j * 128:2 * D + (j + 1) * 128]
                    x1_v[j, pl.ds(mo(HALO + r0 + hf * HM, 16), HM), :] = xx + ga * c[hf * 2 + sd]

    def block(fn):
        pl.when(zero_s[0] == 0)(fn)

    dz = zero_s[0]
    start_up(0)
    c_cp.wait()
    sc16 = silu_c()
    for j in range(4):
        mod_chunk(j, sc16)
    x_cp(0).wait()
    ln1(0, 0)
    k_v[:, 0:HALO, :] = jnp.zeros((8, HALO, 128), F32)
    prep_w(0)
    w_cp(1).wait()
    qkv(0, 0, range(0, 4))
    prep_w(1, wait=False)
    w_cp(2).wait()
    qkv(0, 0, range(4, 8))
    prep_w(2, wait=False)

    def tile(k):
        i = k + (zero_s[0] + 7) % 7
        return i, mo(i * T, T)

    @block
    def _():
        start_up(1)
        x_cp(1).wait()
        i, r0 = tile(0)
        qkv(r0, i, range(8, 12))
        ln1(r0 + T, i + 1)

    @block
    def _():
        x_cp(2).wait()
        wo_cp().wait()
        i, r0 = tile(1)
        v_v[:, 0:HALO, :] = jnp.broadcast_to(v_v[:, HALO:HALO + 1, :], (8, HALO, 128))
        qkv(r0, i)
        qkred(r0 - T, first=True)
        ln1(r0 + T, i + 1)
        prep_wo()

    @block
    def _():
        start_up(2)
        x_cp(3).wait()
        wm_cp(4).wait()
        wm_cp(5).wait()
        i, r0 = tile(2)
        sc = silu_c()
        mod_chunk(4, sc, wait=False)
        mod_chunk(5, sc, wait=False)
        qkv(r0, i)
        sm(r0 - 2 * T)
        qkred(r0 - T)
        ln1(r0 + T, i + 1)

    for i in range(4, NT):
        x_cp(i).wait()

    def mid_body(it, carry):
        @pl.when(it == 0)
        def _():
            start_up(3)
            for j in range(4):
                start_dn(j)

        @pl.when(it == 1)
        def _():
            start_up(4)
            for j in range(6, 12):
                wm_cp(j).start()

        up_grp_wait(it).wait()

        @pl.when(it == 2)
        def _():
            for j in range(4):
                dn_grp(j).wait()

        i = 3 + it % 5
        r0 = mo(i * T, T)
        toks = qkv(r0, i)
        pv(r0 - 3 * T)
        wo(r0 - 3 * T)
        sm(r0 - 2 * T)
        qkred(r0 - T)
        ln1(mo(jnp.minimum(r0 + T, S - T), T), i + 1)
        pieces = 6 * 4 + 5 * 4
        tk = [toks[8 + (len(toks) - 9) * n // pieces] for n in range(pieces)]
        for n in range(6):
            prep_up((i - 3) * 6 + n, tk[4 * n:4 * n + 4])
        for n in range(5):
            prep_dn(jnp.where(i >= 5, 5 * (i - 5) + n, NFT // 2), tk[24 + 4 * n:28 + 4 * n])
        return carry

    lax.fori_loop(0, 5, mid_body, 0)

    @block
    def _():
        for j in range(6, 12):
            wm_cp(j).wait()
        i, r0 = tile(8)
        sc = silu_c()
        for j in range(6, 12):
            mod_chunk(j, sc, wait=False)
        pv(r0 - 3 * T)
        wo(r0 - 3 * T)
        sm(r0 - 2 * T)
        qkred(r0 - T)

    @block
    def _():
        i, r0 = tile(9)
        pv(r0 - 3 * T)
        wo(r0 - 3 * T)
        sm(r0 - 2 * T)
        ln2(r0 - 9 * T, i - 9)

    @block
    def _():
        i, r0 = tile(10)
        ln2(r0 - 9 * T, i - 9)
        pv(r0 - 3 * T)
        wo(r0 - 3 * T)

    def out_cp(r0, r):
        return pltpu.make_async_copy(x_v.at[pl.ds(r0, T), :], out_hbm.at[pl.ds(r0, T), :], sem.at[48 + r])

    def ffn_body(rr, carry):
        r = 2 * rr
        r0 = mo(r * T, T)

        def up(it, c2):
            h = it % 7
            toks = []
            for n in range(2):
                cpair = h * 2 + n
                acts = []
                for nt in (2 * cpair, 2 * cpair + 1):
                    m = []
                    for i in range(7):
                        acc = None
                        for kt in range(4):
                            t = _nn(_bf(jnp.concatenate([sa_v[r, i, kt], sa_v[r + 1, i, kt]], axis=0)), _bf(tu_v[nt, i, kt * 64:(kt + 1) * 64, :]))
                            acc = t if acc is None else acc + t
                        m.append(acc)
                    toks += m
                    gt, ut, gb, ub = _c_blocks(m)
                    acts.append((gt * jax.nn.sigmoid(gt) * ut, gb * jax.nn.sigmoid(gb) * ub))
                (a11, a21), (a12, a22) = acts
                ops = _a_ops(a11, a12, a21, a22)
                for i in range(7):
                    act_b[i, cpair] = ops[i].astype(BF16)
            return c2

        def down(it, c2):
            h = it % 4
            toks = []
            for n in range(1):
                j = h
                m = []
                for i in range(7):
                    acc = None
                    for cpair in range(NFT // 2):
                        t = _nn(_bf(act_v[i, cpair]), _bf(td_v[i, j, cpair]))
                        acc = t if acc is None else acc + t
                    m.append(acc)
                toks += m
                c = _c_blocks(m)
                for hf, u in ((0, 0), (0, 1), (1, 0), (1, 1)):
                    for sd in range(2):
                        jj = j + 4 * sd
                        co = pl.ds(mo(jj * 128, 128), 128)
                        gb = mod_v[0:1, pl.ds(mo(5 * D + jj * 128, 128), 128)]
                        res = x1_v[jj, pl.ds(mo(HALO + r0 + u * T + hf * HM, 16), HM), :] + gb * c[hf * 2 + sd][u * HM:(u + 1) * HM]
                        x_v[pl.ds(mo(r0 + u * T + hf * HM, HM), HM), co] = res.astype(BF16)
            tn = jnp.minimum(r + 2 + h // 2, NT - 1)
            slot = jnp.where(r + 2 < NT, tn, NT)
            for n in range(2):
                b = mo((h % 2) * (2 * LB) + n * LB, LB)
                hs = []
                for ro in (0, HM):
                    cols = [x1_v[q, pl.ds(mo(HALO + tn * T + ro + b, 16), LB), :] for q in range(8)]
                    cols[0] = after(toks[1 + 2 * n + ro // HM], cols[0])
                    hs.append(_layernorm(jnp.concatenate(cols, axis=1)) * modp(4) + modp(3))
                ops = _a_ops(hs[0][:, :512], hs[0][:, 512:], hs[1][:, :512], hs[1][:, 512:])
                for i in range(7):
                    for kt in range(4):
                        sa_b[slot, i, kt, pl.ds(b, LB), :] = ops[i][:, kt * 128:(kt + 1) * 128].astype(BF16)
            return c2

        lax.fori_loop(0, 7, up, 0)
        lax.fori_loop(0, 4, down, 0)
        out_cp(r0, r).start()
        out_cp(r0 + T, r + 1).start()
        return carry

    lax.fori_loop(0, NT // 2, ffn_body, 0)
    for r in range(NT):
        out_cp(r * T, r).wait()


@jax.jit
def pallas_adaLN_cond__sliding_local_dilated__glu_gated_swiglu__prompt_kernel(
    A_x, A_wqkv, A_wo, B_x, B_w1, B_w3, B_w2, c, w_mod,
):
    del B_x
    any_spec = pl.BlockSpec(memory_space=pl.ANY)
    scratch = [
        pltpu.VMEM((8, 6 * D), F32),
        pltpu.VMEM((7, 4, HM, 128), BF16),
        pltpu.VMEM((NT + 1, 7, 4, HM, 128), BF16),
        pltpu.VMEM((12, 7, 4, 128, 128), BF16),
        pltpu.VMEM((7, 4, 512, 128), BF16),
        pltpu.VMEM((8, S, 128), F32),
        pltpu.VMEM((8, S + HALO, 128), F32),
        pltpu.VMEM((8, S + HALO, 128), F32),
        pltpu.VMEM((S, D), BF16),
        pltpu.VMEM((7, NFT // 2, 2 * HM, 128), BF16),
        pltpu.VMEM((NFT + 2, 7, 512, 128), BF16),
        pltpu.VMEM((7, 4, NFT // 2 + 1, 128, 128), BF16),
        pltpu.VMEM((1, D), BF16),
        pltpu.VMEM((12, D, 512), BF16),
        pltpu.VMEM((3, D, D), BF16),
        pltpu.VMEM((8, D, 128), BF16),
        pltpu.VMEM((8, D, 128), BF16),
        pltpu.SemaphoreType.DMA((64,)),
    ]
    out = pl.pallas_call(
        _kernel,
        out_shape=jax.ShapeDtypeStruct((S, D), BF16),
        in_specs=[pl.BlockSpec(memory_space=pltpu.SMEM)] + [any_spec] * 8,
        out_specs=any_spec,
        scratch_shapes=scratch,
        compiler_params=pltpu.CompilerParams(vmem_limit_bytes=126 * 1024 * 1024),
    )(jnp.zeros((1,), I32), A_x.reshape(S, D), A_wqkv, A_wo, B_w1, B_w3, B_w2.reshape(NFT // 2, 2, 128, D), c, w_mod)
    return out.reshape(1, S, D)
```
